```python
import jax
import jax.numpy as jnp

def _softmax(x, axis=-1):
    return jax.nn.softmax(x, axis=axis)
def _gelu(x):
    return jax.nn.gelu(x, approximate=True)
def _silu(x):
    return jax.nn.silu(x)
def _sigmoid(x):
    return jax.nn.sigmoid(x)
def _layernorm(x, axis=-1, eps=1e-5):
    m = jnp.mean(x, axis=axis, keepdims=True)
    v = jnp.var(x, axis=axis, keepdims=True)
    return (x - m) / jnp.sqrt(v + eps)
def _scatter_add(tgt, idx, src, axis=0):
    return tgt.at[idx].add(src)
def _segment_sum(src, seg, n):
    return jax.ops.segment_sum(src, seg, n)
class _Rng:
    def __init__(self, key):
        self._k = key
    def _next(self):
        self._k, sub = jax.random.split(self._k)
        return sub
    def normal(self, shape):
        return jax.random.normal(self._next(), shape, dtype=jnp.bfloat16)
    def randint(self, lo, hi, shape):
        return jax.random.randint(self._next(), shape, lo, hi, dtype=jnp.int32)
    def uniform(self, shape, lo=0.0, hi=1.0):
        return jax.random.uniform(self._next(), shape, jnp.bfloat16, lo, hi)
    def permutation(self, n):
        return jax.random.permutation(self._next(), n)


kernel_name = 'recurrent_scan__ssm_conv_h3__mixer_token_mlp__prompt'

def setup_inputs():
    _rng = _Rng(jax.random.key(int.from_bytes(__import__("os").urandom(4), "little")))
    _w = (lambda a: (lambda t: t.astype(jnp.bfloat16) if jnp.issubdtype(t.dtype, jnp.floating) else t)(jnp.asarray(a)))
    def _A_setup():
        B, S, D = 1, 2048, 576
        ks = 4
        return {
            "q": _w((lambda *s: _rng.normal(s) * 0.05)(B, S, D)),
            "k": _w((lambda *s: _rng.normal(s) * 0.05)(B, S, D)),
            "v": _w((lambda *s: _rng.normal(s) * 0.05)(B, S, D)),
            "shift_k": _w((lambda *s: _rng.normal(s) * 0.05)(D, ks) * 0.5),
            "ssm_k": _w((lambda *s: _rng.normal(s) * 0.05)(D, S) * (1.0 / S ** 0.5)),
            "ssm_D": _w((lambda *s: _rng.normal(s) * 0.05)(D)),
        }
    _A_in = _A_setup()

    def _B_setup():
        B, S, D, F = 1, 2048, 576, 4608
        return {
            "x": _w((lambda *s: _rng.normal(s) * 0.05)(B, S, D)),
            "w1": _w((lambda *s: _rng.normal(s) * 0.05)(S, F) * (S ** -0.5)),
            "b1": _w((lambda *s: _rng.normal(s) * 0.05)(F) * 0.02),
            "w2": _w((lambda *s: _rng.normal(s) * 0.05)(F, S) * (F ** -0.5)),
            "b2": _w((lambda *s: _rng.normal(s) * 0.05)(S) * 0.02),
        }
    _B_in = _B_setup()

    return {
        "A_q": _A_in["q"],
        "A_k": _A_in["k"],
        "A_v": _A_in["v"],
        "A_shift_k": _A_in["shift_k"],
        "A_ssm_k": _A_in["ssm_k"],
        "A_ssm_D": _A_in["ssm_D"],
        "B_x": _B_in["x"],
        "B_w1": _B_in["w1"],
        "B_b1": _B_in["b1"],
        "B_w2": _B_in["w2"],
        "B_b2": _B_in["b2"],
    }

def reference(A_q, A_k, A_v, A_shift_k, A_ssm_k, A_ssm_D, B_x, B_w1, B_b1, B_w2, B_b2):
    def _A_ref(q, k, v, shift_k, ssm_k, ssm_D):
        B, S, D = q.shape
        ks = shift_k.shape[-1]
        k_pad = jnp.pad(k, ((0, 0), (ks - 1, 0), (0, 0)))
        k_shift = jnp.zeros_like(k)
        for t in range(ks):
            k_shift = k_shift + k_pad[:, t:t + S, :] * shift_k[:, ks - 1 - t][None, None, :]
        kv = k_shift * v
        L = 2 * S
        kv_pad = jnp.pad(kv, ((0, 0), (0, S), (0, 0)))
        kf_pad = jnp.pad(ssm_k, ((0, 0), (0, S)))
        kv_f = (lambda x, axes=(-2,-1): jnp.fft.rfft2(x.astype(jnp.float32), axes=axes))(kv_pad[:, None, :, :], axes=(1, 2))
        kf_f = (lambda x, axes=(-2,-1): jnp.fft.rfft2(x.astype(jnp.float32), axes=axes))(kf_pad[:, None, :], axes=(1, 2))
        kf_f = (lambda x, *d: x.transpose(*d))(kf_f, 1, 2, 0)
        y_f = kv_f * kf_f[None, :, :, :]
        y = (lambda x, s, axes=(-2,-1): jnp.fft.irfft2(x, s=s, axes=axes).astype(jnp.bfloat16))(y_f, (1, L), axes=(1, 2))[:, 0, :S, :]
        y = y + kv * ssm_D[None, None, :]
        return q * y

    def _B_ref(x, w1, b1, w2, b2):
        B, S, D = x.shape
        h = _layernorm(x, axis=-1)
        u = jnp.einsum("bsd,sf->bdf", h, w1) + b1
        u = _gelu(u)
        y = jnp.einsum("bdf,fs->bds", u, w2) + b2
        return (lambda x, *d: x.transpose(*d))(y, 0, 2, 1)

    x = A_q
    xn = _layernorm(x, axis=-1)
    s = _A_ref(xn, A_k, A_v, A_shift_k, A_ssm_k, A_ssm_D)
    g = _silu(_B_ref(xn, B_w1, B_b1, B_w2, B_b2))
    return x + s * g
```

```python
import numpy as np
import jax
import jax.numpy as jnp
from jax.experimental import pallas as pl
from jax.experimental.pallas import tpu as pltpu

S, D, F = 2048, 576, 4608
L = 128
NB = S // L
NF = 9
TF = F // NF
SPLIT = 1280
CG = D // NF
f32 = jnp.float32
bf16 = jnp.bfloat16

def _dft_consts():
    n = np.arange(L, dtype=np.float64)[:, None]
    k = np.arange(L, dtype=np.float64)[None, :]
    th = 2.0 * np.pi * n * (k + 0.5) / (2 * L)
    Fm = np.concatenate([np.cos(th), -np.sin(th)], axis=1)
    G = Fm.T / L
    return Fm.astype(jnp.bfloat16), G.astype(jnp.bfloat16)

_FM, _GM = _dft_consts()

def _ln_cols(x):
    m = jnp.mean(x, axis=0, keepdims=True)
    xc = x - m
    v = jnp.mean(xc * xc, axis=0, keepdims=True)
    return xc * jax.lax.rsqrt(v + 1e-5)

def _gelu(u):
    return jax.nn.gelu(u, approximate=True)

def kernel(q_hbm, k_hbm, v_hbm, sk_ref, h_hbm, d_ref, fm_ref, gm_ref, w1_hbm, b1_ref, w2_hbm, b2_ref,
           o_hbm,
           x_ref, hT_ref, xnT_ref, sT_ref, acc_ref, u_ref, w1_buf, w2_buf, k_buf, v_buf, h_buf,
           col_ref, kv_ref, pool_ref, z_ref, o_buf, b1f_ref,
           sem_x, sem_w1, sem_w2, sem_k, sem_v, sem_h, sem_o):

    def w1_copy(t, slot):
        return pltpu.make_async_copy(w1_hbm.at[:, pl.ds(pl.multiple_of(t * TF, TF), TF)], w1_buf.at[slot], sem_w1.at[slot])
    def w2_copy(t, slot):
        return pltpu.make_async_copy(w2_hbm.at[pl.ds(pl.multiple_of(t * TF, TF), TF), :], w2_buf.at[slot], sem_w2.at[slot])
    def kv_copies(g, slot):
        r = pl.ds(pl.multiple_of(g * CG, CG), CG)
        return (pltpu.make_async_copy(k_hbm.at[r, :], k_buf.at[slot], sem_k.at[slot]),
                pltpu.make_async_copy(v_hbm.at[r, :], v_buf.at[slot], sem_v.at[slot]))
    def h_copy(g, slot):
        r = pl.ds(pl.multiple_of(g * CG, CG), CG)
        return pltpu.make_async_copy(h_hbm.at[r, :], h_buf.at[slot], sem_h.at[slot])
    NXC = 4
    XC = S // NXC
    def x_copy(c):
        return pltpu.make_async_copy(q_hbm.at[:, c * XC:(c + 1) * XC], x_ref.at[:, c * XC:(c + 1) * XC], sem_x.at[c])

    for cp in kv_copies(0, 0):
        cp.start()
    h_copy(0, 0).start()
    for c in range(NXC):
        x_copy(c).start()
    w1_copy(0, 0).start()
    for cp in kv_copies(1, 1):
        cp.start()

    skt = sk_ref[...].astype(f32)
    drow = d_ref[...].astype(f32)
    for j in range(4):
        col_ref[j] = jnp.broadcast_to(skt[j:j + 1, :], (128, D)).T
    col_ref[4] = jnp.broadcast_to(drow, (128, D)).T
    fm = fm_ref[...]
    b1v = b1_ref[...].astype(f32)
    for t in range(NF):
        b1f_ref[t] = b1v[t:t + 1, :]
    lane = jax.lax.broadcasted_iota(jnp.int32, (1, L), 1)
    sgn = jnp.where(lane % 2 == 0, 1.0, -1.0).astype(f32)
    lane_s = jax.lax.broadcasted_iota(jnp.int32, (CG, S), 1)

    def make_kv(g, slot):
        gc = jnp.minimum(g, NF - 1)
        r = pl.ds(pl.multiple_of(gc * CG, CG), CG)
        kg = k_buf[slot].astype(f32)
        acc = kg * jnp.tile(col_ref[0, r, :], (1, NB))
        for j in range(1, 4):
            sh = jnp.where(lane_s < j, 0.0, pltpu.roll(kg, j, 1))
            acc = acc + sh * jnp.tile(col_ref[j, r, :], (1, NB))
        kv = (acc * v_buf[slot].astype(f32)).astype(bf16)
        for j in range(NB):
            kv_ref[g, j * CG:(j + 1) * CG, :] = kv[:, j * L:(j + 1) * L]

    def dft(g, slot, xs):
        hg = h_buf[slot]
        lh = jnp.concatenate([hg[:, j * L:(j + 1) * L] for j in range(NB)], axis=0)
        H = jnp.dot(lh, fm, preferred_element_type=f32)
        X = jnp.dot(kv_ref[g], fm, preferred_element_type=f32)
        Hr = H[:, :L]; Hi = H[:, L:]
        pool_ref[xs * 4 + 2, 0:CG, :] = Hr[0:CG]
        pool_ref[xs * 4 + 3, 0:CG, :] = Hi[0:CG]
        pool_ref[xs * 4 + 2, CG:, :] = Hr[CG:] - sgn * Hi[:-CG]
        pool_ref[xs * 4 + 3, CG:, :] = Hi[CG:] + sgn * Hr[:-CG]
        pool_ref[xs * 4] = X[:, :L]
        pool_ref[xs * 4 + 1] = X[:, L:]

    POOL = "1" == "1"
    AH = int("4")
    def spectral_piece(zs, rb, xs, dz=0):
        RB = 8
        def blk(c, j):
            return pool_ref[xs * 4 + c, j * CG + rb * RB:j * CG + (rb + 1) * RB, :]
        for a0 in range(0, NB, AH):
            zr = [None] * AH; zi = [None] * AH
            for j in range(a0 + AH):
                xr = blk(0, j); xi = blk(1, j)
                for a in range(max(a0, j), a0 + AH):
                    hr = blk(2, a - j); hi = blk(3, a - j)
                    q = a - a0
                    if zr[q] is None:
                        zr[q] = xr * hr - xi * hi; zi[q] = xr * hi + xi * hr
                    else:
                        zr[q] = zr[q] + xr * hr - xi * hi; zi[q] = zi[q] + xr * hi + xi * hr
            for q in range(AH):
                a = a0 + q
                rows = slice(a * CG + rb * RB, a * CG + (rb + 1) * RB)
                pool_ref[8 + dz, rows, :] = zr[q]
                pool_ref[9 + dz, rows, :] = zi[q]

    def spectral_pack(zs, lo, hi, dz=0):
        for a in range(NB):
            rows = slice(a * CG + lo, a * CG + hi)
            z_ref[zs, rows, 0:L] = pool_ref[8 + dz, rows, :].astype(bf16)
            z_ref[zs, rows, L:2 * L] = pool_ref[9 + dz, rows, :].astype(bf16)

    def conv_finish(g, zs):
        g = jnp.maximum(g, 0)
        r = pl.ds(pl.multiple_of(g * CG, CG), CG)
        Y = jnp.dot(z_ref[zs], gm_ref[...], preferred_element_type=f32)
        dcol = col_ref[4, r, :]
        xn = xnT_ref[r, :]
        for a in range(NB):
            ya = Y[a * CG:(a + 1) * CG, :] + dcol * kv_ref[g, a * CG:(a + 1) * CG, :].astype(f32)
            sT_ref[r, a * L:(a + 1) * L] = (ya * xn[:, a * L:(a + 1) * L].astype(f32)).astype(bf16)

    def mm1(t, slot):
        u = jnp.dot(hT_ref[...], w1_buf[slot], preferred_element_type=f32)
        return u

    def mm1c(t, slot, c, nc):
        w = TF // nc
        return jnp.dot(hT_ref[...], w1_buf[slot, :, c * w:(c + 1) * w], preferred_element_type=f32)

    def actc(t, slot, u, c, nc):
        w = TF // nc
        b = b1f_ref[t, :, c * w:(c + 1) * w]
        u_ref[slot, :, c * w:(c + 1) * w] = _gelu(u + b).astype(bf16)

    def mm2c(slot, c):
        cs = slice(c * 256, (c + 1) * 256)
        acc_ref[:, cs] += jnp.dot(u_ref[slot], w2_buf[slot, :, cs], preferred_element_type=f32)

    def act(t, slot, u):
        b = b1f_ref[t]
        u_ref[slot] = _gelu(u + b).astype(bf16)

    with jax.named_scope("prologue"):
        for cp in kv_copies(0, 0):
            cp.wait()
        make_kv(0, 0)
        h_copy(0, 0).wait()
        dft(0, 0, 0)
        h_copy(1, 1).start()
        z_ref[1] = jnp.zeros((NB * CG, 2 * L), bf16)
        TC = 128
        for c in range(NXC):
            x_copy(c).wait()
            for cc in range(XC // TC):
                c0 = c * XC + cc * TC
                xt = x_ref[:, c0:c0 + TC].astype(f32)
                xn = _ln_cols(xt).astype(bf16)
                xnT_ref[:, c0:c0 + TC] = xn
                hT_ref[:, c0:c0 + TC] = _ln_cols(xn.astype(f32)).astype(bf16)
            if c == 0:
                w1_copy(1, 1).start()
            if c == 1:
                w2_copy(0, 0).start()
        for cp in kv_copies(1, 1):
            cp.wait()
        for cp in kv_copies(2, 0):
            cp.start()
        w1_copy(0, 0).wait()
        u0 = mm1c(0, 0, 0, 2)
        make_kv(1, 1)
        u1 = mm1c(0, 0, 1, 2)
        actc(0, 0, u0, 0, 2)
        acc_ref[...] = jnp.broadcast_to(b2_ref[...].astype(f32), (D, S))
        actc(0, 0, u1, 1, 2)
        for cp in kv_copies(2, 0):
            cp.wait()
        w1_copy(1, 1).wait()
        h_copy(1, 1).wait()
        w2_copy(0, 0).wait()

    def body(i, carry):
        slot = i % 2
        nslot = 1 - slot
        @pl.when(i + 3 < NF)
        def _():
            for cp in kv_copies(i + 3, nslot):
                cp.start()
        @pl.when(i + 2 < NF)
        def _():
            w1_copy(i + 2, slot).start()
            h_copy(i + 2, slot).start()
        w2_copy(i + 1, nslot).start()
        dz = jax.lax.shift_right_logical(i, 4) if POOL else 0
        sp = lambda rb: spectral_piece(slot, rb, slot, dz)
        pk = lambda lo: spectral_pack(slot, lo, lo + 16, dz)
        sched = "A0.g0.D.B0.s0.B1.s1.p0.B2.s2.B3.s3.p1.F.B4.s4.B5.s5.p2.K.B6.s6.s7.p3.B7"
        N1 = int("1")
        us = {}
        for tok in sched.split("."):
            if tok == "D": dft(i + 1, nslot, nslot)
            elif tok == "F": conv_finish(i - 1, nslot)
            elif tok == "K": make_kv(i + 2, slot)
            elif tok[0] == "A": us[int(tok[1:])] = mm1c(i + 1, nslot, int(tok[1:]), N1)
            elif tok[0] == "g": actc(i + 1, nslot, us[int(tok[1:])], int(tok[1:]), N1)
            elif tok[0] == "s": sp(int(tok[1:]))
            elif tok[0] == "p": pk(16 * int(tok[1:]))
            elif tok[0] == "B": mm2c(slot, int(tok[1:]))
            else: raise ValueError(tok)
        w2_copy(i + 1, nslot).wait()
        @pl.when(i + 3 < NF)
        def _():
            for cp in kv_copies(i + 3, nslot):
                cp.wait()
        @pl.when(i + 2 < NF)
        def _():
            w1_copy(i + 2, slot).wait()
            h_copy(i + 2, slot).wait()
        return carry
    with jax.named_scope("loop"):
        jax.lax.fori_loop(0, NF - 1, body, 0)

    G8 = NF - 1
    LS = G8 % 2
    NOC = 8
    OC = S // NOC
    def ocopy(c):
        cs = slice(c * OC, (c + 1) * OC)
        return pltpu.make_async_copy(o_buf.at[:, cs], o_hbm.at[:, cs], sem_o.at[c])
    def fin_mm(c):
        cs = slice(c * OC, (c + 1) * OC)
        y = acc_ref[:, cs] + jnp.dot(u_ref[LS], w2_buf[LS, :, cs], preferred_element_type=f32)
        return y * jax.nn.sigmoid(y)
    def fin_out(c, g):
        cs = slice(c * OC, (c + 1) * OC)
        o_buf[:, cs] = (x_ref[:, cs].astype(f32) + g * sT_ref[:, cs].astype(f32)).astype(bf16)
        ocopy(c).start()
    def fin_g(c):
        cs = slice(c * OC, (c + 1) * OC)
        acc_ref[:, cs] = fin_mm(c)
    def fin_out2(c):
        cs = slice(c * OC, (c + 1) * OC)
        fin_out(c, acc_ref[:, cs])
    with jax.named_scope("final"):
        sp = lambda rb: spectral_piece(LS, rb, LS)
        pk = lambda lo: spectral_pack(LS, lo, lo + 16)
        conv_finish(G8 - 1, 1 - LS)
        fin_g(0); sp(0); sp(1); pk(0)
        fin_g(1); sp(2); sp(3); pk(16)
        fin_g(2); sp(4); sp(5); pk(32)
        fin_g(3); sp(6); sp(7); pk(48)
        conv_finish(G8, LS)
        g4 = fin_mm(4)
        fin_out2(0); fin_out2(1)
        fin_out(4, g4)
        g5 = fin_mm(5)
        fin_out2(2); fin_out2(3)
        fin_out(5, g5)
        fin_out(6, fin_mm(6))
        fin_out(7, fin_mm(7))
        for c in range(NOC):
            ocopy(c).wait()


@jax.jit
def pallas_recurrent_scan__ssm_conv_h3__mixer_token_mlp__prompt_kernel(
        A_q, A_k, A_v, A_shift_k, A_ssm_k, A_ssm_D, B_x, B_w1, B_b1, B_w2, B_b2):
    qT = A_q[0].T; kT = A_k[0].T; vT = A_v[0].T
    anyspec = pl.BlockSpec(memory_space=pl.ANY)
    vm = pl.BlockSpec(memory_space=pltpu.VMEM)
    out = pl.pallas_call(
        kernel,
        in_specs=[anyspec, anyspec, anyspec, vm, anyspec, vm, vm, vm, anyspec, vm, anyspec, vm],
        out_specs=anyspec,
        out_shape=jax.ShapeDtypeStruct((D, S), bf16),
        scratch_shapes=[pltpu.VMEM((D, S), bf16), pltpu.VMEM((D, S), bf16), pltpu.VMEM((D, S), bf16),
                        pltpu.VMEM((D, S), bf16), pltpu.VMEM((D, S), f32), pltpu.VMEM((2, D, TF), bf16),
                        pltpu.VMEM((2, S, TF), bf16), pltpu.VMEM((2, TF, S), bf16),
                        pltpu.VMEM((2, CG, S), bf16), pltpu.VMEM((2, CG, S), bf16), pltpu.VMEM((2, CG, S), bf16),
                        pltpu.VMEM((5, D, 128), f32), pltpu.VMEM((NF + 1, NB * CG, L), bf16),
                        pltpu.VMEM((10, NB * CG, L), f32),
                        pltpu.VMEM((2, NB * CG, 2 * L), bf16), pltpu.VMEM((D, S), bf16), pltpu.VMEM((NF, 1, TF), f32),
                        pltpu.SemaphoreType.DMA((4,)), pltpu.SemaphoreType.DMA((2,)), pltpu.SemaphoreType.DMA((2,)),
                        pltpu.SemaphoreType.DMA((2,)), pltpu.SemaphoreType.DMA((2,)), pltpu.SemaphoreType.DMA((2,)),
                        pltpu.SemaphoreType.DMA((8,))],
        compiler_params=pltpu.CompilerParams(vmem_limit_bytes=100 * 1024 * 1024),
    )(qT, kT, vT, A_shift_k.T, A_ssm_k, A_ssm_D.reshape(1, D), _FM, _GM, B_w1, B_b1.reshape(NF, TF), B_w2, B_b2.reshape(1, S))
    return out.T[None]
```

```python
import numpy as np
import jax
import jax.numpy as jnp
from jax.experimental import pallas as pl
from jax.experimental.pallas import tpu as pltpu

S, D, F = 2048, 576, 4608
L = 128
NB = S // L
NF = 9
TF = F // NF
SPLIT = 1280
CG = D // NF
f32 = jnp.float32
bf16 = jnp.bfloat16

def _dft_consts():
    n = np.arange(L, dtype=np.float64)[:, None]
    k = np.arange(L, dtype=np.float64)[None, :]
    th = 2.0 * np.pi * n * (k + 0.5) / (2 * L)
    Fm = np.concatenate([np.cos(th), -np.sin(th)], axis=1)
    G = Fm.T / L
    return Fm.astype(jnp.bfloat16), G.astype(jnp.bfloat16)

_FM, _GM = _dft_consts()

def _ln_cols(x):
    m = jnp.mean(x, axis=0, keepdims=True)
    xc = x - m
    v = jnp.mean(xc * xc, axis=0, keepdims=True)
    return xc * jax.lax.rsqrt(v + 1e-5)

def _gelu(u):
    return jax.nn.gelu(u, approximate=True)

def kernel(q_hbm, k_hbm, v_hbm, sk_ref, h_hbm, d_ref, fm_ref, gm_ref, w1_hbm, b1_ref, w2_hbm, b2_ref,
           o_hbm,
           x_ref, hT_ref, xnT_ref, sT_ref, acc_ref, u_ref, w1_buf, w2_buf, k_buf, v_buf, h_buf,
           col_ref, kv_ref, pool_ref, z_ref, o_buf, b1f_ref, uraw_ref,
           sem_x, sem_w1, sem_w2, sem_k, sem_v, sem_h, sem_o):

    def w1_copy(t, slot):
        return pltpu.make_async_copy(w1_hbm.at[:, pl.ds(pl.multiple_of(t * TF, TF), TF)], w1_buf.at[slot], sem_w1.at[slot])
    def w2_copy(t, slot):
        return pltpu.make_async_copy(w2_hbm.at[pl.ds(pl.multiple_of(t * TF, TF), TF), :], w2_buf.at[slot], sem_w2.at[slot])
    def kv_copies(g, slot):
        r = pl.ds(pl.multiple_of(g * CG, CG), CG)
        return (pltpu.make_async_copy(k_hbm.at[r, :], k_buf.at[slot], sem_k.at[slot]),
                pltpu.make_async_copy(v_hbm.at[r, :], v_buf.at[slot], sem_v.at[slot]))
    def h_copy(g, slot):
        r = pl.ds(pl.multiple_of(g * CG, CG), CG)
        return pltpu.make_async_copy(h_hbm.at[r, :], h_buf.at[slot], sem_h.at[slot])
    NXC = 4
    def w1k_copy(c):
        rows = slice(c * (S // NXC), (c + 1) * (S // NXC))
        return pltpu.make_async_copy(w1_hbm.at[rows, 0:TF], w1_buf.at[0, rows, :], sem_x.at[NXC + c])
    XC = S // NXC
    def x_copy(c):
        return pltpu.make_async_copy(q_hbm.at[:, c * XC:(c + 1) * XC], x_ref.at[:, c * XC:(c + 1) * XC], sem_x.at[c])

    for cp in kv_copies(0, 0):
        cp.start()
    h_copy(0, 0).start()
    x_copy(0).start()

    skt = sk_ref[...].astype(f32)
    drow = d_ref[...].astype(f32).reshape(1, D)
    for j in range(4):
        col_ref[j] = jnp.broadcast_to(skt[j:j + 1, :], (128, D)).T
    col_ref[4] = jnp.broadcast_to(drow, (128, D)).T
    fm = fm_ref[...]
    b1v = b1_ref[...].astype(f32).reshape(1, F)
    for t in range(NF):
        b1f_ref[t] = b1v[:, t * TF:(t + 1) * TF]
    lane = jax.lax.broadcasted_iota(jnp.int32, (1, L), 1)
    sgn = jnp.where(lane % 2 == 0, 1.0, -1.0).astype(f32)
    lane_s = jax.lax.broadcasted_iota(jnp.int32, (CG, S), 1)

    def make_kv(g, slot):
        gc = jnp.minimum(g, NF - 1)
        r = pl.ds(pl.multiple_of(gc * CG, CG), CG)
        kg = k_buf[slot].astype(f32)
        acc = kg * jnp.tile(col_ref[0, r, :], (1, NB))
        for j in range(1, 4):
            sh = jnp.where(lane_s < j, 0.0, pltpu.roll(kg, j, 1))
            acc = acc + sh * jnp.tile(col_ref[j, r, :], (1, NB))
        kv = (acc * v_buf[slot].astype(f32)).astype(bf16)
        for j in range(NB):
            kv_ref[g, j * CG:(j + 1) * CG, :] = kv[:, j * L:(j + 1) * L]

    def dft(g, slot, xs):
        hg = h_buf[slot]
        lh = jnp.concatenate([hg[:, j * L:(j + 1) * L] for j in range(NB)], axis=0)
        H = jnp.dot(lh, fm, preferred_element_type=f32)
        X = jnp.dot(kv_ref[g], fm, preferred_element_type=f32)
        Hr = H[:, :L]; Hi = H[:, L:]
        pool_ref[xs * 4 + 2, 0:CG, :] = Hr[0:CG]
        pool_ref[xs * 4 + 3, 0:CG, :] = Hi[0:CG]
        pool_ref[xs * 4 + 2, CG:, :] = Hr[CG:] - sgn * Hi[:-CG]
        pool_ref[xs * 4 + 3, CG:, :] = Hi[CG:] + sgn * Hr[:-CG]
        pool_ref[xs * 4] = X[:, :L]
        pool_ref[xs * 4 + 1] = X[:, L:]

    POOL = "1" == "1"
    AH = int("4")
    def spectral_piece(zs, rb, xs, dz=0):
        RB = 8
        def blk(c, j):
            return pool_ref[xs * 4 + c, j * CG + rb * RB:j * CG + (rb + 1) * RB, :]
        for a0 in range(0, NB, AH):
            zr = [None] * AH; zi = [None] * AH
            for j in range(a0 + AH):
                xr = blk(0, j); xi = blk(1, j)
                for a in range(max(a0, j), a0 + AH):
                    hr = blk(2, a - j); hi = blk(3, a - j)
                    q = a - a0
                    if zr[q] is None:
                        zr[q] = xr * hr - xi * hi; zi[q] = xr * hi + xi * hr
                    else:
                        zr[q] = zr[q] + xr * hr - xi * hi; zi[q] = zi[q] + xr * hi + xi * hr
            for q in range(AH):
                a = a0 + q
                rows = slice(a * CG + rb * RB, a * CG + (rb + 1) * RB)
                pool_ref[8 + dz, rows, :] = zr[q]
                pool_ref[9 + dz, rows, :] = zi[q]

    def spectral_pack(zs, lo, hi, dz=0):
        for a in range(NB):
            rows = slice(a * CG + lo, a * CG + hi)
            z_ref[zs, rows, 0:L] = pool_ref[8 + dz, rows, :].astype(bf16)
            z_ref[zs, rows, L:2 * L] = pool_ref[9 + dz, rows, :].astype(bf16)

    def conv_finish(g, zs):
        r = pl.ds(pl.multiple_of(g * CG, CG), CG)
        Y = jnp.dot(z_ref[zs], gm_ref[...], preferred_element_type=f32)
        dcol = col_ref[4, r, :]
        xn = xnT_ref[r, :]
        for a in range(NB):
            ya = Y[a * CG:(a + 1) * CG, :] + dcol * kv_ref[g, a * CG:(a + 1) * CG, :].astype(f32)
            sT_ref[r, a * L:(a + 1) * L] = (ya * xn[:, a * L:(a + 1) * L].astype(f32)).astype(bf16)

    def mm1(t, slot):
        u = jnp.dot(hT_ref[...], w1_buf[slot], preferred_element_type=f32)
        return u

    def mm1c(t, slot, c, nc):
        w = TF // nc
        return jnp.dot(hT_ref[...], w1_buf[slot, :, c * w:(c + 1) * w], preferred_element_type=f32)

    def actc(t, slot, u, c, nc):
        w = TF // nc
        b = b1f_ref[t, :, c * w:(c + 1) * w]
        u_ref[slot, :, c * w:(c + 1) * w] = _gelu(u + b).astype(bf16)

    def mm2c(slot, c):
        cs = slice(c * 256, (c + 1) * 256)
        acc_ref[:, cs] += jnp.dot(u_ref[slot], w2_buf[slot, :, cs], preferred_element_type=f32)

    def act(t, slot, u):
        b = b1f_ref[t]
        u_ref[slot] = _gelu(u + b).astype(bf16)

    with jax.named_scope("prologue"):
        TC = 128
        def ln(c):
            for cc in range(XC // TC):
                c0 = c * XC + cc * TC
                xt = x_ref[:, c0:c0 + TC].astype(f32)
                xn = _ln_cols(xt).astype(bf16)
                xnT_ref[:, c0:c0 + TC] = xn
                hT_ref[:, c0:c0 + TC] = _ln_cols(xn.astype(f32)).astype(bf16)
        def mmk(c):
            part = jnp.dot(hT_ref[:, c * XC:(c + 1) * XC], w1_buf[0, c * XC:(c + 1) * XC, :], preferred_element_type=f32)
            if c == 0:
                uraw_ref[...] = part
            elif c < NXC - 1:
                uraw_ref[...] += part
            else:
                actc(0, 0, uraw_ref[...] + part, 0, 1)
        for cp in kv_copies(0, 0):
            cp.wait()
        h_copy(0, 0).wait()
        x_copy(1).start(); w1k_copy(0).start()
        make_kv(0, 0)
        dft(0, 0, 0)
        x_copy(0).wait()
        x_copy(2).start(); w1k_copy(1).start()
        ln(0)
        x_copy(1).wait(); w1k_copy(0).wait()
        x_copy(3).start(); w1k_copy(2).start()
        for cp in kv_copies(1, 1):
            cp.start()
        h_copy(1, 1).start()
        mmk(0)
        ln(1)
        x_copy(2).wait(); w1k_copy(1).wait()
        w1k_copy(3).start()
        w1_copy(1, 1).start()
        mmk(1)
        ln(2)
        x_copy(3).wait(); w1k_copy(2).wait()
        for cp in kv_copies(1, 1):
            cp.wait()
        for cp in kv_copies(2, 0):
            cp.start()
        w2_copy(0, 0).start()
        mmk(2)
        ln(3)
        make_kv(1, 1)
        w1k_copy(3).wait()
        w1_copy(1, 1).wait()
        h_copy(1, 1).wait()
        mmk(3)
        acc_ref[...] = jnp.broadcast_to(b2_ref[...].astype(f32).reshape(1, S), (D, S))

    def step(i, slot, nslot, sched, dz):
        sp = lambda rb: spectral_piece(slot, rb, slot, dz)
        pk = lambda lo: spectral_pack(slot, lo, lo + 16, dz)
        N1 = int("1")
        us = {}
        for tok in sched.split("."):
            if tok == "D": dft(i + 1, nslot, nslot)
            elif tok == "F": conv_finish(i - 1, nslot)
            elif tok == "K": make_kv(i + 2, slot)
            elif tok[0] == "A": us[int(tok[1:])] = mm1c(i + 1, nslot, int(tok[1:]), N1)
            elif tok[0] == "g": actc(i + 1, nslot, us[int(tok[1:])], int(tok[1:]), N1)
            elif tok[0] == "s": sp(int(tok[1:]))
            elif tok[0] == "p": pk(16 * int(tok[1:]))
            elif tok[0] == "B": mm2c(slot, int(tok[1:]))
            elif tok == "W":
                w2_copy(0, 0).wait()
                for cp in kv_copies(2, 0):
                    cp.wait()
            else: raise ValueError(tok)

    SCH = "A0.g0.D.B0.s0.B1.s1.p0.B2.s2.B3.s3.p1.F.B4.s4.B5.s5.p2.K.B6.s6.s7.p3.B7"
    with jax.named_scope("it0"):
        for cp in kv_copies(3, 1):
            cp.start()
        h_copy(2, 0).start()
        w1_copy(2, 0).start()
        w2_copy(1, 1).start()
        SCH0 = ".".join(t for t in SCH.replace(".D.", ".D.W.", 1).split(".") if t != "F")
        step(0, 0, 1, SCH0, 0)
        w2_copy(1, 1).wait(); w1_copy(2, 0).wait()
        for cp in kv_copies(3, 1):
            cp.wait()
        h_copy(2, 0).wait()

    def body(i, carry):
        slot = i % 2
        nslot = 1 - slot
        @pl.when(i + 3 < NF)
        def _():
            for cp in kv_copies(i + 3, nslot):
                cp.start()
        @pl.when(i + 2 < NF)
        def _():
            h_copy(i + 2, slot).start()
            w1_copy(i + 2, slot).start()
        w2_copy(i + 1, nslot).start()
        step(i, slot, nslot, SCH, jax.lax.shift_right_logical(i, 4))
        w2_copy(i + 1, nslot).wait()
        @pl.when(i + 3 < NF)
        def _():
            for cp in kv_copies(i + 3, nslot):
                cp.wait()
        @pl.when(i + 2 < NF)
        def _():
            h_copy(i + 2, slot).wait()
            w1_copy(i + 2, slot).wait()
        return i + 1
    with jax.named_scope("loop"):
        ilast = jax.lax.fori_loop(1, NF - 1, body, 1)

    G8 = NF - 1
    LS = G8 % 2
    NOC = 8
    OC = S // NOC
    def ocopy(c):
        cs = slice(c * OC, (c + 1) * OC)
        return pltpu.make_async_copy(o_buf.at[:, cs], o_hbm.at[:, cs], sem_o.at[c])
    def fin_mm(c):
        cs = slice(c * OC, (c + 1) * OC)
        y = acc_ref[:, cs] + jnp.dot(u_ref[LS], w2_buf[LS, :, cs], preferred_element_type=f32)
        hy = 0.5 * y
        return hy * jnp.tanh(hy) + hy
    def fin_out(c, g):
        cs = slice(c * OC, (c + 1) * OC)
        o_buf[:, cs] = (x_ref[:, cs].astype(f32) + g * sT_ref[:, cs].astype(f32)).astype(bf16)
        ocopy(c).start()
    def fin_g(c):
        cs = slice(c * OC, (c + 1) * OC)
        acc_ref[:, cs] = fin_mm(c)
    def fin_out2(c):
        cs = slice(c * OC, (c + 1) * OC)
        fin_out(c, acc_ref[:, cs])
    with jax.named_scope("final"):
        dz = jax.lax.shift_right_logical(ilast, 4)
        gv = {}
        for tok in "G0.s0.s1.p0.F7.G1.s2.s3.p1.G2.s4.s5.p2.G3.s6.s7.p3.F8.M4.O0.O1.o4.M5.O2.O3.o5.M6.o6.M7.o7".split("."):
            k = int(tok[1:])
            if tok[0] == "G": fin_g(k)
            elif tok[0] == "s": spectral_piece(LS, k, LS, dz)
            elif tok[0] == "p": spectral_pack(LS, 16 * k, 16 * k + 16, dz)
            elif tok[0] == "F": conv_finish(k, k % 2)
            elif tok[0] == "M": gv[k] = fin_mm(k)
            elif tok[0] == "O": fin_out2(k)
            elif tok[0] == "o": fin_out(k, gv[k])
            else: raise ValueError(tok)
        for c in range(NOC):
            ocopy(c).wait()


@jax.jit
def pallas_recurrent_scan__ssm_conv_h3__mixer_token_mlp__prompt_kernel(
        A_q, A_k, A_v, A_shift_k, A_ssm_k, A_ssm_D, B_x, B_w1, B_b1, B_w2, B_b2):
    qT = A_q.reshape(S, D).T; kT = A_k.reshape(S, D).T; vT = A_v.reshape(S, D).T
    anyspec = pl.BlockSpec(memory_space=pl.ANY)
    vm = pl.BlockSpec(memory_space=pltpu.VMEM)
    out = pl.pallas_call(
        kernel,
        in_specs=[anyspec, anyspec, anyspec, vm, anyspec, vm, vm, vm, anyspec, vm, anyspec, vm],
        out_specs=anyspec,
        out_shape=jax.ShapeDtypeStruct((D, S), bf16),
        scratch_shapes=[pltpu.VMEM((D, S), bf16), pltpu.VMEM((D, S), bf16), pltpu.VMEM((D, S), bf16),
                        pltpu.VMEM((D, S), bf16), pltpu.VMEM((D, S), f32), pltpu.VMEM((2, D, TF), bf16),
                        pltpu.VMEM((2, S, TF), bf16), pltpu.VMEM((2, TF, S), bf16),
                        pltpu.VMEM((2, CG, S), bf16), pltpu.VMEM((2, CG, S), bf16), pltpu.VMEM((2, CG, S), bf16),
                        pltpu.VMEM((5, D, 128), f32), pltpu.VMEM((NF + 1, NB * CG, L), bf16),
                        pltpu.VMEM((10, NB * CG, L), f32),
                        pltpu.VMEM((2, NB * CG, 2 * L), bf16), pltpu.VMEM((D, S), bf16), pltpu.VMEM((NF, 1, TF), f32), pltpu.VMEM((D, TF), f32),
                        pltpu.SemaphoreType.DMA((8,)), pltpu.SemaphoreType.DMA((2,)), pltpu.SemaphoreType.DMA((2,)),
                        pltpu.SemaphoreType.DMA((2,)), pltpu.SemaphoreType.DMA((2,)), pltpu.SemaphoreType.DMA((2,)),
                        pltpu.SemaphoreType.DMA((8,))],
        compiler_params=pltpu.CompilerParams(vmem_limit_bytes=100 * 1024 * 1024),
    )(qT, kT, vT, A_shift_k.T, A_ssm_k, A_ssm_D, _FM, _GM, B_w1, B_b1, B_w2, B_b2)
    return out.T.reshape(1, S, D)
```

```python
import numpy as np
import jax
import jax.numpy as jnp
from jax.experimental import pallas as pl
from jax.experimental.pallas import tpu as pltpu

S, D, F = 2048, 576, 4608
L = 128
NB = S // L
NF = 9
TF = F // NF
SPLIT = 1280
CG = D // NF
f32 = jnp.float32
bf16 = jnp.bfloat16

def _dft_consts():
    n = np.arange(L, dtype=np.float64)[:, None]
    k = np.arange(L, dtype=np.float64)[None, :]
    th = 2.0 * np.pi * n * (k + 0.5) / (2 * L)
    Fm = np.concatenate([np.cos(th), -np.sin(th)], axis=1)
    G = Fm.T / L
    return Fm.astype(jnp.bfloat16), G.astype(jnp.bfloat16)

_FM, _GM = _dft_consts()
_Z0 = np.zeros((1,), np.int32)

def _tree(lst):
    while len(lst) > 1:
        nl = [lst[i] + lst[i + 1] for i in range(0, len(lst) - 1, 2)]
        if len(lst) % 2:
            nl.append(lst[-1])
        lst = nl
    return lst[0]

def _colmean(x):
    if "0" == "0":
        return jnp.mean(x, axis=0, keepdims=True)
    n, _ = x.shape
    t = _tree([x[i * 72:(i + 1) * 72] for i in range(n // 72)])
    t = _tree([t[j * 8:(j + 1) * 8] for j in range(9)])
    return jnp.sum(t, axis=0, keepdims=True) * (1.0 / n)

def _ln_cols(x):
    m = _colmean(x)
    xc = x - m
    v = _colmean(xc * xc)
    return xc * jax.lax.rsqrt(v + 1e-5)

def _gelu(u):
    return jax.nn.gelu(u, approximate=True)

def kernel(zero_ref, q_hbm, k_hbm, v_hbm, sk_ref, h_hbm, d_ref, fm_ref, gm_ref, w1_hbm, b1_ref, w2_hbm, b2_ref,
           o_hbm,
           x_ref, hT_ref, xnT_ref, sT_ref, acc_ref, u_ref, w1_buf, w2_buf, k_buf, v_buf, h_buf,
           col_ref, kv_ref, pool_ref, z_ref, o_buf, b1f_ref, uraw_ref, ha_ref, hb_ref,
           sem_x, sem_w1, sem_w2, sem_k, sem_v, sem_h, sem_o):

    def w1_copy(t, slot):
        return pltpu.make_async_copy(w1_hbm.at[:, pl.ds(pl.multiple_of(t * TF, TF), TF)], w1_buf.at[slot], sem_w1.at[slot])
    def w2_copy(t, slot):
        return pltpu.make_async_copy(w2_hbm.at[pl.ds(pl.multiple_of(t * TF, TF), TF), :], w2_buf.at[slot], sem_w2.at[slot])
    def kv_copies(g, slot):
        r = pl.ds(pl.multiple_of(g * CG, CG), CG)
        return (pltpu.make_async_copy(k_hbm.at[r, :], k_buf.at[slot], sem_k.at[slot]),
                pltpu.make_async_copy(v_hbm.at[r, :], v_buf.at[slot], sem_v.at[slot]))
    def h_copy(g, slot):
        r = pl.ds(pl.multiple_of(g * CG, CG), CG)
        return pltpu.make_async_copy(h_hbm.at[r, :], h_buf.at[slot], sem_h.at[slot])
    XO = [int(t) for t in "0.256.768.1280.1792.2048".split(".")]
    NXC = len(XO) - 1
    def w1k_copy(c):
        rows = slice(XO[c], XO[c + 1])
        return pltpu.make_async_copy(w1_hbm.at[rows, 0:TF], w1_buf.at[0, rows, :], sem_x.at[NXC + c])
    def x_copy(c):
        return pltpu.make_async_copy(q_hbm.at[:, XO[c]:XO[c + 1]], x_ref.at[:, XO[c]:XO[c + 1]], sem_x.at[c])

    for cp in kv_copies(0, 0):
        cp.start()
    h_copy(0, 0).start()
    x_copy(0).start()

    skt = sk_ref[...].astype(f32)
    drow = d_ref[...].astype(f32).reshape(1, D)
    for j in range(4):
        col_ref[j] = jnp.broadcast_to(skt[j:j + 1, :], (128, D)).T
    col_ref[4] = jnp.broadcast_to(drow, (128, D)).T
    fm = fm_ref[...]
    b1v = b1_ref[...].astype(f32).reshape(1, F)
    for t in range(NF):
        b1f_ref[t] = b1v[:, t * TF:(t + 1) * TF]
    lane = jax.lax.broadcasted_iota(jnp.int32, (1, L), 1)
    sgn = jnp.where(lane % 2 == 0, 1.0, -1.0).astype(f32)

    def make_kv(g, slot, part=0, nparts=1):
        gc = jnp.minimum(g, NF - 1)
        R = CG // nparts
        r = pl.ds(pl.multiple_of(gc * CG + part * R, R), R)
        rs = slice(part * R, (part + 1) * R)
        lane_s = jax.lax.broadcasted_iota(jnp.int32, (R, S), 1)
        kg = k_buf[slot, rs, :].astype(f32)
        acc = kg * jnp.tile(col_ref[0, r, :], (1, NB))
        for j in range(1, 4):
            sh = jnp.where(lane_s < j, 0.0, pltpu.roll(kg, j, 1))
            acc = acc + sh * jnp.tile(col_ref[j, r, :], (1, NB))
        kv = (acc * v_buf[slot, rs, :].astype(f32)).astype(bf16)
        for j in range(NB):
            kv_ref[g, j * CG + part * R:j * CG + (part + 1) * R, :] = kv[:, j * L:(j + 1) * L]

    def dft(g, slot, xs):
        hg = h_buf[slot]
        lh = jnp.concatenate([hg[:, j * L:(j + 1) * L] for j in range(NB)], axis=0)
        H = jnp.dot(lh, fm, preferred_element_type=f32)
        X = jnp.dot(kv_ref[g], fm, preferred_element_type=f32)
        Hr = H[:, :L]; Hi = H[:, L:]
        pool_ref[xs * 4 + 2, 0:CG, :] = Hr[0:CG]
        pool_ref[xs * 4 + 3, 0:CG, :] = Hi[0:CG]
        pool_ref[xs * 4 + 2, CG:, :] = Hr[CG:] - sgn * Hi[:-CG]
        pool_ref[xs * 4 + 3, CG:, :] = Hi[CG:] + sgn * Hr[:-CG]
        pool_ref[xs * 4] = X[:, :L]
        pool_ref[xs * 4 + 1] = X[:, L:]

    POOL = "1" == "1"
    AH = int("2")
    def spectral_piece(zs, rb, xs, dz=0):
        RB = 8
        def blk(c, j):
            return pool_ref[xs * 4 + c, j * CG + rb * RB:j * CG + (rb + 1) * RB, :]
        for a0 in range(0, NB, AH):
            zr = [None] * AH; zi = [None] * AH
            for j in range(a0 + AH):
                xr = blk(0, j); xi = blk(1, j)
                for a in range(max(a0, j), a0 + AH):
                    hr = blk(2, a - j); hi = blk(3, a - j)
                    q = a - a0
                    if zr[q] is None:
                        zr[q] = xr * hr - xi * hi; zi[q] = xr * hi + xi * hr
                    else:
                        zr[q] = zr[q] + xr * hr - xi * hi; zi[q] = zi[q] + xr * hi + xi * hr
            for q in range(AH):
                a = a0 + q
                rows = slice(a * CG + rb * RB, a * CG + (rb + 1) * RB)
                pool_ref[8 + dz, rows, :] = zr[q]
                pool_ref[9 + dz, rows, :] = zi[q]

    def spectral_pack(zs, lo, hi, dz=0):
        for a in range(NB):
            rows = slice(a * CG + lo, a * CG + hi)
            z_ref[zs, rows, 0:L] = pool_ref[8 + dz, rows, :].astype(bf16)
            z_ref[zs, rows, L:2 * L] = pool_ref[9 + dz, rows, :].astype(bf16)

    def conv_finish(g, zs):
        r = pl.ds(pl.multiple_of(g * CG, CG), CG)
        Y = jnp.dot(z_ref[zs], gm_ref[...], preferred_element_type=f32)
        dcol = col_ref[4, r, :]
        xn = xnT_ref[r, :]
        for a in range(NB):
            ya = Y[a * CG:(a + 1) * CG, :] + dcol * kv_ref[g, a * CG:(a + 1) * CG, :].astype(f32)
            sT_ref[r, a * L:(a + 1) * L] = (ya * xn[:, a * L:(a + 1) * L].astype(f32)).astype(bf16)

    def mm1(t, slot):
        u = jnp.dot(hT_ref[...], w1_buf[slot], preferred_element_type=f32)
        return u

    def mm1c(t, slot, c, nc):
        w = TF // nc
        return jnp.dot(hT_ref[...], w1_buf[slot, :, c * w:(c + 1) * w], preferred_element_type=f32)

    def actc(t, slot, u, c, nc):
        w = TF // nc
        b = b1f_ref[t, :, c * w:(c + 1) * w]
        u_ref[slot, :, c * w:(c + 1) * w] = _gelu(u + b).astype(bf16)

    def mm2c(slot, c, first=False):
        cs = slice(c * 256, (c + 1) * 256)
        d = jnp.dot(u_ref[slot], w2_buf[slot, :, cs], preferred_element_type=f32)
        if first:
            acc_ref[:, cs] = d + b2_ref[...].astype(f32).reshape(1, S)[:, cs]
        else:
            acc_ref[:, cs] += d

    def act(t, slot, u):
        b = b1f_ref[t]
        u_ref[slot] = _gelu(u + b).astype(bf16)

    with jax.named_scope("prologue"):
        TC = 128
        HAB = "0" == "1"
        def ln(c):
            for c0 in range(XO[c], XO[c + 1], TC):
                xt = x_ref[:, c0:c0 + TC].astype(f32)
                xn = _ln_cols(xt).astype(bf16)
                xnT_ref[:, c0:c0 + TC] = xn
                hh = _ln_cols(xn.astype(f32)).astype(bf16)
                hT_ref[:, c0:c0 + TC] = hh
                if HAB:
                    (ha_ref, hb_ref)[c % 2][:, c0 - XO[c]:c0 - XO[c] + TC] = hh
        def mmk(c):
            part = jnp.dot((ha_ref, hb_ref)[c % 2][:, 0:XO[c + 1] - XO[c]] if HAB else hT_ref[:, XO[c]:XO[c + 1]], w1_buf[0, XO[c]:XO[c + 1], :], preferred_element_type=f32)
            if c == 0:
                uraw_ref[...] = part
            elif c < NXC - 1:
                uraw_ref[...] += part
            else:
                actc(0, 0, uraw_ref[...] + part, 0, 1)
        for cp in kv_copies(0, 0):
            cp.wait()
        h_copy(0, 0).wait()
        w1k_copy(0).start()
        x_copy(1).start()
        make_kv(0, 0)
        dft(0, 0, 0)
        x_copy(0).wait()
        w1k_copy(1).start(); x_copy(2).start()
        ln(0)
        for c in range(NXC):
            w1k_copy(c).wait()
            if c + 1 < NXC:
                x_copy(c + 1).wait()
            if c + 2 < NXC:
                w1k_copy(c + 2).start()
            if c + 3 < NXC:
                x_copy(c + 3).start()
            if c == 1:
                for cp in kv_copies(1, 1):
                    cp.start()
                h_copy(1, 1).start()
            if c == NXC - 3:
                w1_copy(1, 1).start()
            if c == NXC - 2:
                for cp in kv_copies(1, 1):
                    cp.wait()
                for cp in kv_copies(2, 0):
                    cp.start()
                w2_copy(0, 0).start()
            if c == NXC - 1:
                w1_copy(1, 1).wait()
                h_copy(1, 1).wait()
            mmk(c)
            if c + 1 < NXC:
                ln(c + 1)
            if c == NXC - 2:
                make_kv(1, 1)

    def step(i, slot, nslot, sched, dz):
        sp = lambda rb: spectral_piece(slot, rb, slot, dz)
        pk = lambda lo: spectral_pack(slot, lo, lo + 16, dz)
        N1 = int("1")
        us = {}
        for tok in sched.split("."):
            if tok == "D": dft(i + 1, nslot, nslot)
            elif tok == "F": conv_finish(i - 1, nslot)
            elif tok == "K": make_kv(i + 2, slot)
            elif tok[0] == "k": make_kv(i + 2, slot, int(tok[1]), int(tok[2]))
            elif tok[0] == "A": us[int(tok[1:])] = mm1c(i + 1, nslot, int(tok[1:]), N1)
            elif tok[0] == "g": actc(i + 1, nslot, us[int(tok[1:])], int(tok[1:]), N1)
            elif tok[0] == "s": sp(int(tok[1:]))
            elif tok[0] == "p": pk(16 * int(tok[1:]))
            elif tok[0] == "B": mm2c(slot, int(tok[1:]))
            elif tok[0] == "b": mm2c(slot, int(tok[1:]), True)
            elif tok == "W":
                w2_copy(0, 0).wait()
                for cp in kv_copies(2, 0):
                    cp.wait()
            else: raise ValueError(tok)

    SCH = "A0.D.g0.B0.s0.s1.p0.B1.s2.s3.p1.B2.s4.s5.p2.B3.s6.s7.p3.F.B4.k04.k14.B5.k24.B6.k34.B7"
    with jax.named_scope("it0"):
        for cp in kv_copies(3, 1):
            cp.start()
        h_copy(2, 0).start()
        w1_copy(2, 0).start()
        w2_copy(1, 1).start()
        SCH0 = "A0.g0.D.W.b0.s0.s1.p0.b1.s2.s3.p1.b2.s4.s5.p2.b3.s6.s7.p3.b4.k02.b5.k12.b6.b7"
        z0 = zero_ref[0]
        step(z0, z0, 1 - z0, SCH0, z0)
        w2_copy(1, 1).wait(); w1_copy(2, 0).wait()
        for cp in kv_copies(3, 1):
            cp.wait()
        h_copy(2, 0).wait()

    def body(i, carry):
        slot = i % 2
        nslot = 1 - slot
        @pl.when(i + 3 < NF)
        def _():
            for cp in kv_copies(i + 3, nslot):
                cp.start()
        @pl.when(i + 2 < NF)
        def _():
            h_copy(i + 2, slot).start()
            w1_copy(i + 2, slot).start()
        w2_copy(i + 1, nslot).start()
        step(i, slot, nslot, SCH, jax.lax.shift_right_logical(i, 4))
        w2_copy(i + 1, nslot).wait()
        @pl.when(i + 3 < NF)
        def _():
            for cp in kv_copies(i + 3, nslot):
                cp.wait()
        @pl.when(i + 2 < NF)
        def _():
            h_copy(i + 2, slot).wait()
            w1_copy(i + 2, slot).wait()
        return i + 1
    with jax.named_scope("loop"):
        ilast = jax.lax.fori_loop(1, NF - 1, body, 1)

    G8 = NF - 1
    LS = G8 % 2
    NOC = 8
    OC = S // NOC
    def ocopy(c):
        cs = slice(c * OC, (c + 1) * OC)
        return pltpu.make_async_copy(o_buf.at[:, cs], o_hbm.at[:, cs], sem_o.at[c])
    def fin_mm(c):
        cs = slice(c * OC, (c + 1) * OC)
        y = acc_ref[:, cs] + jnp.dot(u_ref[LS], w2_buf[LS, :, cs], preferred_element_type=f32)
        hy = 0.5 * y
        return hy * jnp.tanh(hy) + hy
    def fin_out(c, g):
        cs = slice(c * OC, (c + 1) * OC)
        o_buf[:, cs] = (x_ref[:, cs].astype(f32) + g * sT_ref[:, cs].astype(f32)).astype(bf16)
        ocopy(c).start()
    def fin_g(c):
        cs = slice(c * OC, (c + 1) * OC)
        acc_ref[:, cs] = fin_mm(c)
    def fin_out2(c):
        cs = slice(c * OC, (c + 1) * OC)
        fin_out(c, acc_ref[:, cs])
    with jax.named_scope("final"):
        dz = jax.lax.shift_right_logical(ilast, 4)
        gv = {}
        for tok in "s0.s1.p0.G0.s2.s3.p1.G1.s4.s5.p2.G2.s6.s7.p3.G3.G4.G5.X4.F7.F8.M6.O0.O1.O2.o6.M7.O3.O4.O5.o7".split("."):
            k = int(tok[1:])
            if tok[0] == "G": fin_g(k)
            elif tok[0] == "s": spectral_piece(LS, k, LS, dz)
            elif tok[0] == "p": spectral_pack(LS, 16 * k, 16 * k + 16, dz)
            elif tok[0] == "F": conv_finish(k, k % 2)
            elif tok[0] == "M": gv[k] = fin_mm(k)
            elif tok[0] == "O": fin_out2(k)
            elif tok[0] == "X":
                z_ref[2 + dz, 0:16, 0:L] = acc_ref[0:16, k * OC:k * OC + L].astype(bf16)
            elif tok[0] == "o": fin_out(k, gv[k])
            else: raise ValueError(tok)
        for c in range(NOC):
            ocopy(c).wait()


@jax.jit
def pallas_recurrent_scan__ssm_conv_h3__mixer_token_mlp__prompt_kernel(
        A_q, A_k, A_v, A_shift_k, A_ssm_k, A_ssm_D, B_x, B_w1, B_b1, B_w2, B_b2):
    qT = A_q.reshape(S, D).T; kT = A_k.reshape(S, D).T; vT = A_v.reshape(S, D).T
    anyspec = pl.BlockSpec(memory_space=pl.ANY)
    vm = pl.BlockSpec(memory_space=pltpu.VMEM)
    out = pl.pallas_call(
        kernel,
        in_specs=[pl.BlockSpec(memory_space=pltpu.SMEM), anyspec, anyspec, anyspec, vm, anyspec, vm, vm, vm, anyspec, vm, anyspec, vm],
        out_specs=anyspec,
        out_shape=jax.ShapeDtypeStruct((D, S), bf16),
        scratch_shapes=[pltpu.VMEM((D, S), bf16), pltpu.VMEM((D, S), bf16), pltpu.VMEM((D, S), bf16),
                        pltpu.VMEM((D, S), bf16), pltpu.VMEM((D, S), f32), pltpu.VMEM((2, D, TF), bf16),
                        pltpu.VMEM((2, S, TF), bf16), pltpu.VMEM((2, TF, S), bf16),
                        pltpu.VMEM((2, CG, S), bf16), pltpu.VMEM((2, CG, S), bf16), pltpu.VMEM((2, CG, S), bf16),
                        pltpu.VMEM((5, D, 128), f32), pltpu.VMEM((NF + 1, NB * CG, L), bf16),
                        pltpu.VMEM((10, NB * CG, L), f32),
                        pltpu.VMEM((3, NB * CG, 2 * L), bf16), pltpu.VMEM((D, S), bf16), pltpu.VMEM((NF, 1, TF), f32), pltpu.VMEM((D, TF), f32), pltpu.VMEM((D, 512), bf16), pltpu.VMEM((D, 512), bf16),
                        pltpu.SemaphoreType.DMA((16,)), pltpu.SemaphoreType.DMA((2,)), pltpu.SemaphoreType.DMA((2,)),
                        pltpu.SemaphoreType.DMA((2,)), pltpu.SemaphoreType.DMA((2,)), pltpu.SemaphoreType.DMA((2,)),
                        pltpu.SemaphoreType.DMA((8,))],
        compiler_params=pltpu.CompilerParams(vmem_limit_bytes=100 * 1024 * 1024),
    )(_Z0, qT, kT, vT, A_shift_k.T, A_ssm_k, A_ssm_D, _FM, _GM, B_w1, B_b1, B_w2, B_b2)
    return out.T.reshape(1, S, D)
```

```python
import numpy as np
import jax
import jax.numpy as jnp
from jax.experimental import pallas as pl
from jax.experimental.pallas import tpu as pltpu

S, D, F = 2048, 576, 4608
L = 128
NB = S // L
NF = 9
TF = F // NF
CG = D // NF
f32 = jnp.float32
bf16 = jnp.bfloat16

def _dft_consts():
    n = np.arange(L, dtype=np.float64)[:, None]
    k = np.arange(L, dtype=np.float64)[None, :]
    th = 2.0 * np.pi * n * (k + 0.5) / (2 * L)
    Fm = np.concatenate([np.cos(th), -np.sin(th)], axis=1)
    G = Fm.T / L
    return Fm.astype(jnp.bfloat16), G.astype(jnp.bfloat16)

_FM, _GM = _dft_consts()
_Z0 = np.zeros((1,), np.int32)

def _ln_cols(x):
    m = jnp.mean(x, axis=0, keepdims=True)
    xc = x - m
    v = jnp.mean(xc * xc, axis=0, keepdims=True)
    return xc * jax.lax.rsqrt(v + 1e-5)

def _gelu(u):
    return jax.nn.gelu(u, approximate=True)

def kernel(zero_ref, q_hbm, k_hbm, v_hbm, sk_ref, h_hbm, d_ref, fm_ref, gm_ref, w1_hbm, b1_ref, w2_hbm, b2_ref,
           o_hbm,
           x_ref, hT_ref, xnT_ref, sT_ref, acc_ref, u_ref, w1_buf, w2_buf, k_buf, v_buf, h_buf,
           col_ref, kv_ref, pool_ref, z_ref, o_buf, b1f_ref, uraw_ref,
           sem_x, sem_w1, sem_w2, sem_k, sem_v, sem_h, sem_o):

    def w1_copy(t, slot):
        return pltpu.make_async_copy(w1_hbm.at[:, pl.ds(pl.multiple_of(t * TF, TF), TF)], w1_buf.at[slot], sem_w1.at[slot])
    def w2_copy(t, slot):
        return pltpu.make_async_copy(w2_hbm.at[pl.ds(pl.multiple_of(t * TF, TF), TF), :], w2_buf.at[slot], sem_w2.at[slot])
    def kv_copies(g, slot):
        r = pl.ds(pl.multiple_of(g * CG, CG), CG)
        return (pltpu.make_async_copy(k_hbm.at[r, :], k_buf.at[slot], sem_k.at[slot]),
                pltpu.make_async_copy(v_hbm.at[r, :], v_buf.at[slot], sem_v.at[slot]))
    def h_copy(g, slot):
        r = pl.ds(pl.multiple_of(g * CG, CG), CG)
        return pltpu.make_async_copy(h_hbm.at[r, :], h_buf.at[slot], sem_h.at[slot])
    XO = [0, 256, 768, 1280, 1792, 2048]
    NXC = len(XO) - 1
    def w1k_copy(c):
        rows = slice(XO[c], XO[c + 1])
        return pltpu.make_async_copy(w1_hbm.at[rows, 0:TF], w1_buf.at[0, rows, :], sem_x.at[NXC + c])
    def x_copy(c):
        return pltpu.make_async_copy(q_hbm.at[:, XO[c]:XO[c + 1]], x_ref.at[:, XO[c]:XO[c + 1]], sem_x.at[c])

    for cp in kv_copies(0, 0):
        cp.start()
    h_copy(0, 0).start()
    x_copy(0).start()

    skt = sk_ref[...].astype(f32)
    drow = d_ref[...].astype(f32).reshape(1, D)
    for j in range(4):
        col_ref[j] = jnp.broadcast_to(skt[j:j + 1, :], (128, D)).T
    col_ref[4] = jnp.broadcast_to(drow, (128, D)).T
    fm = fm_ref[...]
    b1v = b1_ref[...].astype(f32).reshape(1, F)
    for t in range(NF):
        b1f_ref[t] = b1v[:, t * TF:(t + 1) * TF]
    lane = jax.lax.broadcasted_iota(jnp.int32, (1, L), 1)
    sgn = jnp.where(lane % 2 == 0, 1.0, -1.0).astype(f32)

    def make_kv(g, slot, part=0, nparts=1):
        gc = jnp.minimum(g, NF - 1)
        R = CG // nparts
        r = pl.ds(pl.multiple_of(gc * CG + part * R, R), R)
        rs = slice(part * R, (part + 1) * R)
        lane_s = jax.lax.broadcasted_iota(jnp.int32, (R, S), 1)
        kg = k_buf[slot, rs, :].astype(f32)
        acc = kg * jnp.tile(col_ref[0, r, :], (1, NB))
        for j in range(1, 4):
            sh = jnp.where(lane_s < j, 0.0, pltpu.roll(kg, j, 1))
            acc = acc + sh * jnp.tile(col_ref[j, r, :], (1, NB))
        kv = (acc * v_buf[slot, rs, :].astype(f32)).astype(bf16)
        for j in range(NB):
            kv_ref[g, j * CG + part * R:j * CG + (part + 1) * R, :] = kv[:, j * L:(j + 1) * L]

    def dft(g, slot, xs):
        hg = h_buf[slot]
        lh = jnp.concatenate([hg[:, j * L:(j + 1) * L] for j in range(NB)], axis=0)
        H = jnp.dot(lh, fm, preferred_element_type=f32)
        X = jnp.dot(kv_ref[g], fm, preferred_element_type=f32)
        Hr = H[:, :L]; Hi = H[:, L:]
        pool_ref[xs * 4 + 2, 0:CG, :] = Hr[0:CG]
        pool_ref[xs * 4 + 3, 0:CG, :] = Hi[0:CG]
        pool_ref[xs * 4 + 2, CG:, :] = Hr[CG:] - sgn * Hi[:-CG]
        pool_ref[xs * 4 + 3, CG:, :] = Hi[CG:] + sgn * Hr[:-CG]
        pool_ref[xs * 4] = X[:, :L]
        pool_ref[xs * 4 + 1] = X[:, L:]

    AH = 2
    def spectral_piece(zs, rb, xs, dz=0):
        RB = 8
        def blk(c, j):
            return pool_ref[xs * 4 + c, j * CG + rb * RB:j * CG + (rb + 1) * RB, :]
        for a0 in range(0, NB, AH):
            zr = [None] * AH; zi = [None] * AH
            for j in range(a0 + AH):
                xr = blk(0, j); xi = blk(1, j)
                for a in range(max(a0, j), a0 + AH):
                    hr = blk(2, a - j); hi = blk(3, a - j)
                    q = a - a0
                    if zr[q] is None:
                        zr[q] = xr * hr - xi * hi; zi[q] = xr * hi + xi * hr
                    else:
                        zr[q] = zr[q] + xr * hr - xi * hi; zi[q] = zi[q] + xr * hi + xi * hr
            for q in range(AH):
                a = a0 + q
                rows = slice(a * CG + rb * RB, a * CG + (rb + 1) * RB)
                pool_ref[8 + dz, rows, :] = zr[q]
                pool_ref[9 + dz, rows, :] = zi[q]

    def spectral_pack(zs, lo, hi, dz=0):
        for a in range(NB):
            rows = slice(a * CG + lo, a * CG + hi)
            z_ref[zs, rows, 0:L] = pool_ref[8 + dz, rows, :].astype(bf16)
            z_ref[zs, rows, L:2 * L] = pool_ref[9 + dz, rows, :].astype(bf16)

    def conv_finish(g, zs):
        r = pl.ds(pl.multiple_of(g * CG, CG), CG)
        Y = jnp.dot(z_ref[zs], gm_ref[...], preferred_element_type=f32)
        dcol = col_ref[4, r, :]
        xn = xnT_ref[r, :]
        for a in range(NB):
            ya = Y[a * CG:(a + 1) * CG, :] + dcol * kv_ref[g, a * CG:(a + 1) * CG, :].astype(f32)
            sT_ref[r, a * L:(a + 1) * L] = (ya * xn[:, a * L:(a + 1) * L].astype(f32)).astype(bf16)

    def mm1c(t, slot, c, nc):
        w = TF // nc
        return jnp.dot(hT_ref[...], w1_buf[slot, :, c * w:(c + 1) * w], preferred_element_type=f32)

    def actc(t, slot, u, c, nc):
        w = TF // nc
        b = b1f_ref[t, :, c * w:(c + 1) * w]
        u_ref[slot, :, c * w:(c + 1) * w] = _gelu(u + b).astype(bf16)

    def mm2c(slot, c, first=False):
        cs = slice(c * 256, (c + 1) * 256)
        d = jnp.dot(u_ref[slot], w2_buf[slot, :, cs], preferred_element_type=f32)
        if first:
            acc_ref[:, cs] = d + b2_ref[...].astype(f32).reshape(1, S)[:, cs]
        else:
            acc_ref[:, cs] += d

    with jax.named_scope("prologue"):
        TC = 128
        W2AT = NXC - 1
        W1AT = NXC - 3
        def ln(c):
            for c0 in range(XO[c], XO[c + 1], TC):
                xt = x_ref[:, c0:c0 + TC].astype(f32)
                xn = _ln_cols(xt).astype(bf16)
                xnT_ref[:, c0:c0 + TC] = xn
                hT_ref[:, c0:c0 + TC] = _ln_cols(xn.astype(f32)).astype(bf16)
        def mmk(c):
            part = jnp.dot(hT_ref[:, XO[c]:XO[c + 1]], w1_buf[0, XO[c]:XO[c + 1], :], preferred_element_type=f32)
            if c == 0:
                uraw_ref[...] = part
            elif c < NXC - 1:
                uraw_ref[...] += part
            else:
                actc(0, 0, uraw_ref[...] + part, 0, 1)
        for cp in kv_copies(0, 0):
            cp.wait()
        h_copy(0, 0).wait()
        w1k_copy(0).start()
        x_copy(1).start()
        make_kv(0, 0)
        dft(0, 0, 0)
        x_copy(0).wait()
        w1k_copy(1).start(); x_copy(2).start()
        ln(0)
        for c in range(NXC):
            w1k_copy(c).wait()
            if c + 1 < NXC:
                x_copy(c + 1).wait()
            if c + 2 < NXC:
                w1k_copy(c + 2).start()
            if c + 3 < NXC:
                x_copy(c + 3).start()
            if c == 1:
                for cp in kv_copies(1, 1):
                    cp.start()
                h_copy(1, 1).start()
            if c == W1AT:
                w1_copy(1, 1).start()
            if c == NXC - 2:
                for cp in kv_copies(1, 1):
                    cp.wait()
            if c == W2AT:
                for cp in kv_copies(2, 0):
                    cp.start()
                w2_copy(0, 0).start()
            if c == NXC - 1:
                w1_copy(1, 1).wait()
                h_copy(1, 1).wait()
            mmk(c)
            if c + 1 < NXC:
                ln(c + 1)
            if c == NXC - 2:
                make_kv(1, 1)

    def step(i, slot, nslot, sched, dz):
        sp = lambda rb: spectral_piece(slot, rb, slot, dz)
        pk = lambda lo: spectral_pack(slot, lo, lo + 16, dz)
        us = {}
        for tok in sched.split("."):
            if tok == "D": dft(i + 1, nslot, nslot)
            elif tok == "F": conv_finish(i - 1, nslot)
            elif tok[0] == "k": make_kv(i + 2, slot, int(tok[1]), int(tok[2]))
            elif tok[0] == "A": us[int(tok[1:])] = mm1c(i + 1, nslot, int(tok[1:]), 1)
            elif tok[0] == "g": actc(i + 1, nslot, us[int(tok[1:])], int(tok[1:]), 1)
            elif tok[0] == "s": sp(int(tok[1:]))
            elif tok[0] == "p": pk(16 * int(tok[1:]))
            elif tok[0] == "B": mm2c(slot, int(tok[1:]))
            elif tok[0] == "b": mm2c(slot, int(tok[1:]), True)
            elif tok == "W":
                w2_copy(0, 0).wait()
                for cp in kv_copies(2, 0):
                    cp.wait()
            else: raise ValueError(tok)

    SCH = "A0.D.g0.B0.s0.s1.p0.B1.s2.s3.p1.B2.s4.s5.p2.B3.s6.s7.p3.F.B4.k04.k14.B5.k24.B6.k34.B7"
    with jax.named_scope("it0"):
        for cp in kv_copies(3, 1):
            cp.start()
        h_copy(2, 0).start()
        w1_copy(2, 0).start()
        w2_copy(1, 1).start()
        SCH0 = "A0.g0.D.W.b0.s0.s1.p0.b1.s2.s3.p1.b2.s4.s5.p2.b3.s6.s7.p3.b4.k02.b5.k12.b6.b7"
        z0 = zero_ref[0]
        step(z0, z0, 1 - z0, SCH0, z0)
        w2_copy(1, 1).wait(); w1_copy(2, 0).wait()
        for cp in kv_copies(3, 1):
            cp.wait()
        h_copy(2, 0).wait()

    def body(i, carry):
        slot = i % 2
        nslot = 1 - slot
        @pl.when(i + 3 < NF)
        def _():
            for cp in kv_copies(i + 3, nslot):
                cp.start()
        @pl.when(i + 2 < NF)
        def _():
            h_copy(i + 2, slot).start()
            w1_copy(i + 2, slot).start()
        w2_copy(i + 1, nslot).start()
        step(i, slot, nslot, SCH, jax.lax.shift_right_logical(i, 4))
        w2_copy(i + 1, nslot).wait()
        @pl.when(i + 3 < NF)
        def _():
            for cp in kv_copies(i + 3, nslot):
                cp.wait()
        @pl.when(i + 2 < NF)
        def _():
            h_copy(i + 2, slot).wait()
            w1_copy(i + 2, slot).wait()
        return i + 1
    with jax.named_scope("loop"):
        ilast = jax.lax.fori_loop(1, NF - 1, body, 1)

    G8 = NF - 1
    LS = G8 % 2
    OCB = [0, 256, 512, 768, 1024, 1280, 1536, 1792, 2048]
    NOC = len(OCB) - 1
    ocs = lambda c: slice(OCB[c], OCB[c + 1])
    def ocopy(c):
        return pltpu.make_async_copy(o_buf.at[:, ocs(c)], o_hbm.at[:, ocs(c)], sem_o.at[c])
    def fin_mm(c):
        y = acc_ref[:, ocs(c)] + jnp.dot(u_ref[LS], w2_buf[LS, :, ocs(c)], preferred_element_type=f32)
        hy = 0.5 * y
        return hy * jnp.tanh(hy) + hy
    def fin_out(c, g):
        o_buf[:, ocs(c)] = (x_ref[:, ocs(c)].astype(f32) + g * sT_ref[:, ocs(c)].astype(f32)).astype(bf16)
        ocopy(c).start()
    def fin_g(c):
        acc_ref[:, ocs(c)] = fin_mm(c)
    def fin_out2(c):
        fin_out(c, acc_ref[:, ocs(c)])
    with jax.named_scope("final"):
        dz = jax.lax.shift_right_logical(ilast, 4)
        gv = {}
        for tok in "s0.s1.p0.G0.s2.s3.p1.G1.s4.s5.p2.G2.s6.s7.p3.G3.G4.G5.X4.F7.F8.M6.O0.O1.O2.o6.M7.O3.O4.O5.o7".split("."):
            k = int(tok[1:])
            if tok[0] == "G": fin_g(k)
            elif tok[0] == "s": spectral_piece(LS, k, LS, dz)
            elif tok[0] == "p": spectral_pack(LS, 16 * k, 16 * k + 16, dz)
            elif tok[0] == "F": conv_finish(k, k % 2)
            elif tok[0] == "M": gv[k] = fin_mm(k)
            elif tok[0] == "O": fin_out2(k)
            elif tok[0] == "X":
                z_ref[2 + dz, 0:16, 0:L] = acc_ref[0:16, OCB[k]:OCB[k] + L].astype(bf16)
            elif tok[0] == "o": fin_out(k, gv[k])
            else: raise ValueError(tok)
        for c in range(NOC):
            ocopy(c).wait()


@jax.jit
def pallas_recurrent_scan__ssm_conv_h3__mixer_token_mlp__prompt_kernel(
        A_q, A_k, A_v, A_shift_k, A_ssm_k, A_ssm_D, B_x, B_w1, B_b1, B_w2, B_b2):
    qT = A_q.reshape(S, D).T; kT = A_k.reshape(S, D).T; vT = A_v.reshape(S, D).T
    anyspec = pl.BlockSpec(memory_space=pl.ANY)
    vm = pl.BlockSpec(memory_space=pltpu.VMEM)
    out = pl.pallas_call(
        kernel,
        in_specs=[pl.BlockSpec(memory_space=pltpu.SMEM), anyspec, anyspec, anyspec, vm, anyspec, vm, vm, vm, anyspec, vm, anyspec, vm],
        out_specs=anyspec,
        out_shape=jax.ShapeDtypeStruct((D, S), bf16),
        scratch_shapes=[pltpu.VMEM((D, S), bf16), pltpu.VMEM((D, S), bf16), pltpu.VMEM((D, S), bf16),
                        pltpu.VMEM((D, S), bf16), pltpu.VMEM((D, S), f32), pltpu.VMEM((2, D, TF), bf16),
                        pltpu.VMEM((2, S, TF), bf16), pltpu.VMEM((2, TF, S), bf16),
                        pltpu.VMEM((2, CG, S), bf16), pltpu.VMEM((2, CG, S), bf16), pltpu.VMEM((2, CG, S), bf16),
                        pltpu.VMEM((5, D, 128), f32), pltpu.VMEM((NF + 1, NB * CG, L), bf16),
                        pltpu.VMEM((10, NB * CG, L), f32),
                        pltpu.VMEM((3, NB * CG, 2 * L), bf16), pltpu.VMEM((D, S), bf16), pltpu.VMEM((NF, 1, TF), f32), pltpu.VMEM((D, TF), f32),
                        pltpu.SemaphoreType.DMA((16,)), pltpu.SemaphoreType.DMA((2,)), pltpu.SemaphoreType.DMA((2,)),
                        pltpu.SemaphoreType.DMA((2,)), pltpu.SemaphoreType.DMA((2,)), pltpu.SemaphoreType.DMA((2,)),
                        pltpu.SemaphoreType.DMA((12,))],
        compiler_params=pltpu.CompilerParams(vmem_limit_bytes=100 * 1024 * 1024),
    )(_Z0, qT, kT, vT, A_shift_k.T, A_ssm_k, A_ssm_D, _FM, _GM, B_w1, B_b1, B_w2, B_b2)
    return out.T.reshape(1, S, D)
```
